```python
import os as _os
_os.environ.setdefault("JAX_PLATFORMS", "cpu")
import jax
import jax.numpy as jnp

def _softmax(x, axis=-1):
    return jax.nn.softmax(x, axis=axis)
def _gelu(x):
    return jax.nn.gelu(x, approximate=True)
def _silu(x):
    return jax.nn.silu(x)
def _sigmoid(x):
    return jax.nn.sigmoid(x)
def _layernorm(x, axis=-1, eps=1e-5):
    m = jnp.mean(x, axis=axis, keepdims=True)
    v = jnp.var(x, axis=axis, keepdims=True)
    return (x - m) / jnp.sqrt(v + eps)
def _scatter_add(tgt, idx, src, axis=0):
    return tgt.at[idx].add(src)
def _segment_sum(src, seg, n):
    return jax.ops.segment_sum(src, seg, n)
class _Rng:
    def __init__(self, key):
        self._k = key
    def _next(self):
        self._k, sub = jax.random.split(self._k)
        return sub
    def normal(self, shape):
        return jax.random.normal(self._next(), shape, dtype=jnp.bfloat16)
    def randint(self, lo, hi, shape):
        return jax.random.randint(self._next(), shape, lo, hi, dtype=jnp.int32)
    def uniform(self, shape, lo=0.0, hi=1.0):
        return jax.random.uniform(self._next(), shape, jnp.bfloat16, lo, hi)
    def permutation(self, n):
        return jax.random.permutation(self._next(), n)


kernel_name = 'gated_mix__ssm_conv_h3__mixer_s_mlp__prompt'

def setup_inputs():
    _rng = _Rng(jax.random.key(int.from_bytes(__import__("os").urandom(4), "little")))
    _w = (lambda a: (lambda t: t.astype(jnp.bfloat16) if jnp.issubdtype(t.dtype, jnp.floating) else t)(jnp.asarray(a)))
    def _A_setup():
        B, S, D = 1, 2048, 576
        ks = 4
        return {
            "q": _w((lambda *s: _rng.normal(s) * 0.05)(B, S, D)),
            "k": _w((lambda *s: _rng.normal(s) * 0.4)(B, S, D)),
            "v": _w((lambda *s: _rng.normal(s) * 0.4)(B, S, D)),
            "shift_k": _w((lambda *s: _rng.normal(s) * 0.4)(D, ks) * 0.5),
            "ssm_k": _w((lambda *s: _rng.normal(s) * 0.4)(D, S) * (1.0 / S ** 0.5)),
            "ssm_D": _w((lambda *s: _rng.normal(s) * 0.4)(D)),
        }
    _A_in = _A_setup()

    def _B_setup():
        B, S, D, F = 1, 2048, 576, 4608
        return {
            "x":  _w((lambda *s: _rng.normal(s) * 0.05)(B, S, D)),
            "w1": _w((lambda *s: _rng.normal(s) * 0.2)(D, D) * (D ** -0.5)),
            "w2": _w((lambda *s: _rng.normal(s) * 0.2)(D, D) * (D ** -0.5)),
            "w3": _w((lambda *s: _rng.normal(s) * 0.2)(D, F) * (D ** -0.5)),
            "w4": _w((lambda *s: _rng.normal(s) * 0.2)(F, D) * (F ** -0.5)),
        }
    _B_in = _B_setup()

    return {
        "A_q": _A_in["q"],
        "A_k": _A_in["k"],
        "A_v": _A_in["v"],
        "A_shift_k": _A_in["shift_k"],
        "A_ssm_k": _A_in["ssm_k"],
        "A_ssm_D": _A_in["ssm_D"],
        "B_x": _B_in["x"],
        "B_w1": _B_in["w1"],
        "B_w2": _B_in["w2"],
        "B_w3": _B_in["w3"],
        "B_w4": _B_in["w4"],
        "gate_w": _w((lambda *s: _rng.normal(s) * 0.05)(576) * 16.0),
    }

def reference(A_q, A_k, A_v, A_shift_k, A_ssm_k, A_ssm_D, B_x, B_w1, B_w2, B_w3, B_w4, gate_w):
    def _A_ref(q, k, v, shift_k, ssm_k, ssm_D):
        B, S, D = q.shape
        ks = shift_k.shape[-1]
        k_pad = jnp.pad(k, ((0, 0), (ks - 1, 0), (0, 0)))
        k_shift = jnp.zeros_like(k)
        for t in range(ks):
            k_shift = k_shift + k_pad[:, t:t + S, :] * shift_k[:, ks - 1 - t][None, None, :]
        kv = k_shift * v
        L = 2 * S
        kv_pad = jnp.pad(kv, ((0, 0), (0, S), (0, 0)))
        kf_pad = jnp.pad(ssm_k, ((0, 0), (0, S)))
        kv_f = (lambda x, axes=(-2,-1): jnp.fft.rfft2(x.astype(jnp.float32), axes=axes))(kv_pad[:, None, :, :], axes=(1, 2))
        kf_f = (lambda x, axes=(-2,-1): jnp.fft.rfft2(x.astype(jnp.float32), axes=axes))(kf_pad[:, None, :], axes=(1, 2))
        kf_f = (lambda x, *d: x.transpose(*d))(kf_f, 1, 2, 0)
        y_f = kv_f * kf_f[None, :, :, :]
        y = (lambda x, s, axes=(-2,-1): jnp.fft.irfft2(x, s=s, axes=axes).astype(jnp.bfloat16))(y_f, (1, L), axes=(1, 2))[:, 0, :S, :]
        y = y + kv * ssm_D[None, None, :]
        return q * y

    def _B_ref(x, w1, w2, w3, w4):
        B, S, D = x.shape
        h = _gelu(_layernorm(x, axis=-1) @ w1)
        c = D // 4
        g0 = jnp.pad(h[:, :, 0*c:1*c], ((0, 0), (1, 0), (0, 0)))[:, :S, :]
        g1 = jnp.pad(h[:, :, 1*c:2*c], ((0, 0), (0, 1), (0, 0)))[:, 1:, :]
        g2 = jnp.pad(h[:, :, 2*c:3*c], ((0, 0), (2, 0), (0, 0)))[:, :S, :]
        g3 = jnp.pad(h[:, :, 3*c:   ], ((0, 0), (0, 2), (0, 0)))[:, 2:, :]
        hs = jnp.concatenate([g0, g1, g2, g3], axis=-1) @ w2
        x1 = x + hs
        h2 = _gelu(_layernorm(x1, axis=-1) @ w3) @ w4
        return x1 + h2

    x = A_q
    g = _sigmoid((x * gate_w).sum(-1, keepdims=True))
    a = _A_ref(x, A_k, A_v, A_shift_k, A_ssm_k, A_ssm_D)
    b = _B_ref(x, B_w1, B_w2, B_w3, B_w4)
    return g * a + (1 - g) * b
```

```python
import numpy as np
import jax
import jax.numpy as jnp
from jax import lax
import jax.experimental.pallas as pl
import jax.experimental.pallas.tpu as pltpu

S, D, F = 2048, 576, 4608
BLK = 128
NB = S // BLK
TF = 512
NF = F // TF
TM = 512
NT = S // TM
TPC = TM // BLK
NU = 6
CU = D // NU
C4 = D // 4
RG = 16
NG = D // RG
KF = 512
W1P = ((0, 256), (256, D))
SHIFTS = (1, -1, 2, -2)

_F32 = jnp.float32
_BF16 = jnp.bfloat16
_U32 = jnp.uint32


def _dft_consts():
    t = np.arange(BLK, dtype=np.float64)[:, None]
    f = np.arange(BLK, dtype=np.float64)[None, :]
    th = np.pi * (2.0 * f + 1.0) * t / (2.0 * BLK)
    fwd = np.concatenate([np.cos(th), -np.sin(th)], axis=1)
    inv = fwd.T / BLK
    return fwd.astype(np.float32), inv.astype(np.float32)


def _gelu(x):
    c = 0.7978845608028654
    t = jnp.tanh(x * (c + (c * 0.044715) * (x * x)))
    hx = 0.5 * x
    return hx + hx * t


def _col_bcast(row):
    return jnp.broadcast_to(row, (128, D)).T


def _fold8(x):
    acc = x[0:8]
    for r in range(1, x.shape[0] // 8):
        acc = acc + x[r * 8:(r + 1) * 8]
    return acc


def _pk(x):
    return pltpu.bitcast(x, _U32)


def _upk(x):
    return pltpu.bitcast(x, _BF16)


class _Side:
    def __init__(self, jobs, nslots):
        self.jobs = []
        for gen, n in jobs:
            next(gen)
            self.jobs.append(gen)
        self.total = sum(n for _, n in jobs)
        self.nslots = nslots
        self.slot = 0
        self.done = 0

    def _one(self, dep):
        try:
            self.jobs[0].send(dep)
        except StopIteration:
            self.jobs.pop(0)
        self.done += 1

    def step(self, dep, weight=1):
        self.slot += weight
        target = min(self.total, -(-self.total * self.slot // self.nslots))
        while self.done < target:
            self._one(dep)

    def finish(self):
        while self.done < self.total:
            self._one(None)
        assert not self.jobs


def _kernel(q_hbm, k_hbm, v_hbm, sk_hbm, w1_hbm, w2_hbm, w3_hbm, w4_hbm,
            sh_hbm, sd_hbm, gw_hbm, fwd_hbm, inv_hbm, o_hbm,
            acc_ref, ga_ref, xn1a_ref, xn1b_ref, xn2_ref, h0_ref, h1_ref, h2_ref, h3_ref, kv_ref, u_ref, kf_ref, z_ref,
            g_ref, col_ref, w1t_ref, w2t_ref,
            q_ref, k_ref, v_ref, sk_ref, w1_ref, w2_ref, w3_ref, w4_ref, o_ref,
            sh_ref, sd_ref, gw_ref, fwd_ref, inv_ref,
            x1l_ref, sem):
    xn1_refs = (xn1a_ref, xn1b_ref)
    h_refs = (h0_ref, h1_ref, h2_ref, h3_ref)

    def copy(src, dst, s):
        return pltpu.make_async_copy(src, dst, sem.at[s])

    def q_copy(c):
        return copy(q_hbm.at[:, pl.ds(c * TM, TM)], q_ref.at[:, pl.ds(c * TM, TM)], (2, 4, 5, 5)[c])

    w1_copies = [copy(w1_hbm.at[r0:r1], w1_ref.at[r0:r1], s) for s, (r0, r1) in zip((1, 3), W1P)]
    w2_copy = copy(w2_hbm, w2_ref, 5)
    par_copies = [copy(sh_hbm, sh_ref, 0), copy(sd_hbm, sd_ref, 0), copy(gw_hbm, gw_ref, 0)]
    dft_copies = [copy(fwd_hbm, fwd_ref, 3), copy(inv_hbm, inv_ref, 3)]

    def w_copies(j):
        cols = pl.ds(j * TF, TF)
        return [copy(w3_hbm.at[:, cols], w3_ref.at[j], 1 + j % 2),
                copy(w4_hbm.at[:, cols], w4_ref.at[j], 1 + j % 2)]

    def c_copies(j):
        rows = pl.ds(j * CU, CU)
        return [copy(k_hbm.at[rows, :], k_ref.at[j], 1 + j % 2),
                copy(v_hbm.at[rows, :], v_ref.at[j], 1 + j % 2),
                copy(sk_hbm.at[rows, :], sk_ref.at[j], 1 + j % 2)]

    o_pieces = [(0, 4, 0, NG), (4, 4, 0, NG), (8, 4, 0, NG), (12, 2, 0, NG), (14, 1, 0, NG),
                (15, 1, 0, 24), (15, 1, 24, NG)]

    def o_copy(i):
        p0, n, g0, g1 = o_pieces[i]
        idx = (pl.ds(g0 * RG, (g1 - g0) * RG), pl.ds(p0 * BLK, n * BLK))
        return copy(o_ref.at[idx], o_hbm.at[idx], 0)

    for cp in par_copies + [w1_copies[0]]:
        cp.start()
    later = ([q_copy(0), w1_copies[1], q_copy(1), q_copy(2), q_copy(3), w2_copy] + dft_copies
             + w_copies(0) + c_copies(0))

    def start_next(n=1):
        for _ in range(n):
            if later:
                later.pop(0).start()

    lane = lax.broadcasted_iota(jnp.int32, (8, BLK), 1)
    sgn = 1.0 - 2.0 * (lane % 2).astype(_F32)
    never = sgn > 2.0
    oz = lax.fori_loop(0, 3, lambda i, c: c * i, 7)

    def pin(x, dep):
        if dep is None:
            return x
        d = dep[0:8]
        if x.dtype != d.dtype:
            d = pltpu.bitcast(d, x.dtype)
        head = jnp.where(never, d, x[0:8])
        return head if x.shape[0] == 8 else jnp.concatenate([head, x[8:]], axis=0)

    def sub_pinned(x, mu8, dep):
        m = pin(mu8, dep)
        return x - jnp.concatenate([m] * (x.shape[0] // 8), axis=0)

    def ln1_job(p):
        cols = slice(p * BLK, (p + 1) * BLK)
        ocols = slice((p % TPC) * BLK, (p % TPC + 1) * BLK)
        R = 2 * RG
        s = None
        for g in range(D // (2 * R)):
            dep = yield
            a = _fold8(pin(q_ref[g * 2 * R:(g + 1) * 2 * R, cols].astype(_F32), dep))
            s = a if s is None else s + a
        mu = jnp.broadcast_to(jnp.sum(s, axis=0, keepdims=True) * (1.0 / D), (8, BLK))
        v = None
        for g in range(D // R):
            dep = yield
            xc = sub_pinned(q_ref[g * R:(g + 1) * R, cols].astype(_F32), mu, dep)
            a = _fold8(xc * xc)
            v = a if v is None else v + a
        rs = lax.rsqrt(jnp.sum(v, axis=0, keepdims=True) * (1.0 / D) + 1e-5)
        for g in range(D // R):
            dep = yield
            xc = sub_pinned(q_ref[g * R:(g + 1) * R, cols].astype(_F32), mu, dep)
            xn1_refs[(p // TPC) % 2][0, g * R:(g + 1) * R, ocols] = xc * rs

    LN1_N = D // (4 * RG) + 2 * (D // (2 * RG))

    def ln2_job(p, s):
        if s is None:
            src, cols = x1l_ref, slice(0, BLK)
            s = x1l_ref[D:D + 8, :]
        else:
            src, cols = acc_ref, slice(p * BLK, (p + 1) * BLK)
        R = 2 * RG
        mu = None
        v = None
        for g in range(D // R):
            dep = yield
            if mu is None:
                mu = jnp.broadcast_to(jnp.sum(s, axis=0, keepdims=True) * (1.0 / D), (8, BLK))
            xc = sub_pinned(src[g * R:(g + 1) * R, cols], mu, dep)
            a = _fold8(xc * xc)
            v = a if v is None else v + a
        rs = lax.rsqrt(jnp.sum(v, axis=0, keepdims=True) * (1.0 / D) + 1e-5)
        for b in range(5):
            dep = yield
            r0, r1 = b * 128, min(D, (b + 1) * 128)
            xc = sub_pinned(src[r0:r1, cols], mu, dep)
            xn2_ref[p * (BLK // 2):(p + 1) * (BLK // 2), r0:r1] = _pk((xc * rs).astype(_BF16).T)

    LN2_N = D // (2 * RG) + 5

    def kv_job(j):
        for g in range(CU // RG):
            rows = slice(g * RG, (g + 1) * RG)
            crow = pl.ds(pl.multiple_of(j * CU + g * RG, RG), RG)
            prev = None
            for b in range(NB):
                dep = yield
                cols = slice(b * BLK, (b + 1) * BLK)
                ku = pin(_pk(k_ref[j, rows, cols]), dep)
                rolled = [pltpu.roll(ku, tau, 1) for tau in range(1, 4)]
                ks = _upk(ku).astype(_F32) * col_ref[0, crow, :]
                for tau in range(1, 4):
                    lo = jnp.zeros_like(ku) if prev is None else prev[tau - 1]
                    sh = _upk(jnp.where(lane < tau, lo, rolled[tau - 1])).astype(_F32)
                    ks = ks + sh * col_ref[tau, crow, :]
                prev = rolled
                kv_ref[0, b, rows, :] = ks * v_ref[j, rows, cols].astype(_F32)

    KV_N = (CU // RG) * NB

    def mac_job():
        for g in range(CU // 8):
            rows = slice(g * 8, (g + 1) * 8)
            yp = None
            for i in range(NB):
                yr = None
                yi = None
                for m in range(i + 1):
                    dep = yield
                    kr = pin(kf_ref[m, rows, 0:BLK], dep)
                    ki = kf_ref[m, rows, BLK:2 * BLK]
                    ur = u_ref[i - m, rows, 0:BLK]
                    ui = u_ref[i - m, rows, BLK:2 * BLK]
                    pr = kr * ur - ki * ui
                    pi = kr * ui + ki * ur
                    yr = pr if yr is None else yr + pr
                    yi = pi if yi is None else yi + pi
                if yp is None:
                    zr, zi = yr, yi
                else:
                    zr = yr - sgn * yp[1]
                    zi = yi + sgn * yp[0]
                yp = (yr, yi)
                z_ref[0, i, rows, 0:BLK] = zr
                z_ref[0, i, rows, BLK:2 * BLK] = zi

    MAC_N = (CU // 8) * (NB * (NB + 1) // 2)

    start_next()
    with jax.named_scope('setup'):
        for cp in par_copies:
            cp.wait()
        start_next()
        col_ref[5] = _col_bcast(gw_ref[...].astype(_F32).reshape(1, D))
        for r in range(4):
            col_ref[r] = _col_bcast(sh_ref[r:r + 1, :].astype(_F32))
        col_ref[4] = _col_bcast(sd_ref[...].astype(_F32).reshape(1, D))
        w1_copies[0].wait()
        start_next()
        w1t_ref[:, W1P[0][0]:W1P[0][1]] = _pk(w1_ref[W1P[0][0]:W1P[0][1], :].T)
    with jax.named_scope('setup2'):
        q_copy(0).wait()
        start_next()
        _Side([(ln1_job(p), LN1_N) for p in range(3)], 1).finish()
    with jax.named_scope('setup3'):
        w1_copies[1].wait()
        start_next(2)
        w1t_ref[:, W1P[1][0]:W1P[1][1]] = _pk(w1_ref[W1P[1][0]:W1P[1][1], :].T)
        _Side([(ln1_job(3), LN1_N)], 1).finish()

    def w_segment(wt_ref, x_tile, c, per_round, epilogue):
        side, wgt, fin = per_round(0)
        xr = jnp.concatenate([x_tile(KF, D, c * TPC + t) for t in range(TPC)], axis=1)
        part = jnp.dot(_upk(wt_ref[:, KF:D]), xr.astype(_BF16), preferred_element_type=_F32)
        for g in range(NG):
            side.step(part[g * RG:(g + 1) * RG, 0:BLK], wgt)
        if fin:
            side.finish()
        for t in range(TPC):
            p = c * TPC + t
            side, wgt, fin = per_round(t + 1)
            r = jnp.dot(_upk(wt_ref[:, 0:KF]), x_tile(0, KF, p).astype(_BF16),
                        preferred_element_type=_F32)
            for g in range(NG):
                rg = r[g * RG:(g + 1) * RG] + part[g * RG:(g + 1) * RG, t * BLK:(t + 1) * BLK]
                epilogue(rg, g, p)
                side.step(rg, wgt)
            if fin:
                side.finish()

    def w1_epilogue(rg, g, p):
        sft = SHIFTS[g * RG // C4]
        h_refs[p // TPC][0, g * RG:(g + 1) * RG, (p % TPC) * BLK:(p % TPC + 1) * BLK] = (
            pltpu.roll(_gelu(rg), sft % BLK, 1))

    def xn1_tile(r0, r1, p):
        return xn1_refs[(p // TPC) % 2][oz, r0:r1, (p % TPC) * BLK:(p % TPC + 1) * BLK]

    def h_tile(r0, r1, p):
        if p < 0 or p >= NB:
            return jnp.zeros((r1 - r0, BLK), _F32)
        return h_refs[p // TPC][oz, r0:r1, (p % TPC) * BLK:(p % TPC + 1) * BLK]

    def hs_tile(r0, r1, p):
        parts = []
        for gi, sft in enumerate(SHIFTS):
            a0, a1 = max(r0, gi * C4), min(r1, (gi + 1) * C4)
            if a0 >= a1:
                continue
            ln = lax.broadcasted_iota(jnp.int32, (a1 - a0, BLK), 1)
            if sft > 0:
                parts.append(jnp.where(ln < sft, h_tile(a0, a1, p - 1), h_tile(a0, a1, p)))
            else:
                parts.append(jnp.where(ln >= BLK + sft, h_tile(a0, a1, p + 1), h_tile(a0, a1, p)))
        return parts[0] if len(parts) == 1 else jnp.concatenate(parts, axis=0)

    with jax.named_scope('w1'):
        for c in range(NT):
            state = {}

            def per_round(rnd, c=c, state=state):
                first = 2 if c < 2 else 0
                if rnd < first or c + 1 == NT:
                    return _Side([], 1), 1, False
                if rnd == first:
                    if c == 0:
                        q_copy(1).wait()
                    if c == 1:
                        start_next(len(later))
                        q_copy(2).wait()
                        q_copy(3).wait()
                        w2_copy.wait()
                    jobs = [(ln1_job((c + 1) * TPC + t), LN1_N) for t in range(TPC)]
                    state['side'] = _Side(jobs, (3 if c < 2 else 6) * NG - 16)
                return state['side'], (2 if rnd == 0 else 1), rnd == TPC

            if c == NT - 1:
                w2t_ref[...] = _pk(w2_ref[...].T)
            w_segment(w1t_ref, xn1_tile, c, per_round, w1_epilogue)

    sums = {}
    gsums = {}

    def w2_epilogue(rg, g, p):
        cols = slice(p * BLK, (p + 1) * BLK)
        x = q_ref[g * RG:(g + 1) * RG, cols].astype(_F32)
        x1 = rg + x
        acc_ref[g * RG:(g + 1) * RG, cols] = x1
        if p == NB - 1:
            x1l_ref[g * RG:(g + 1) * RG, :] = x1
        a = _fold8(x1)
        b = _fold8(x * col_ref[5, g * RG:(g + 1) * RG, :])
        sums[p] = a if g == 0 else sums[p] + a
        gsums[p] = b if g == 0 else gsums[p] + b
        if g == NG - 1:
            gate = jax.nn.sigmoid(jnp.sum(gsums.pop(p), axis=0, keepdims=True))
            g_ref[:, cols] = jnp.broadcast_to(gate, (8, BLK))

    with jax.named_scope('w2'):
        for c in range(NT):
            def per_round(rnd, c=c):
                pprev = c * TPC + rnd - 2 if rnd >= 2 else c * TPC - 1 if rnd == 0 else -1
                jobs = [(ln2_job(pprev, sums.pop(pprev)), LN2_N)] if pprev >= 0 else []
                return _Side(jobs, NG), 1, True
            w_segment(w2t_ref, hs_tile, c, per_round, w2_epilogue)
        x1l_ref[D:D + 8, :] = sums.pop(NB - 1)
        assert not later
        for cp in dft_copies:
            cp.wait()

    def mlp_tile(j, t, side, last=False):
        xn = _upk(xn2_ref[t * (TM // 2):(t + 1) * (TM // 2), :])
        h = jnp.dot(xn, w3_ref[j], preferred_element_type=_F32)
        h = _gelu(h).astype(_BF16)
        w4 = w4_ref[j]
        for pp in range(TPC):
            p = t * TPC + pp
            cols = slice(p * BLK, (p + 1) * BLK)
            r = lax.dot_general(w4, h[pp * BLK:(pp + 1) * BLK], (((1,), (1,)), ((), ())),
                                preferred_element_type=_F32)
            for g in range(NG):
                rows = slice(g * RG, (g + 1) * RG)
                rg = r[rows]
                a = acc_ref[rows, cols] + rg
                acc_ref[rows, cols] = a
                if last:
                    omg = 1.0 - g_ref[0:1, cols]
                    o_ref[rows, cols] = (ga_ref[rows, cols] + omg * a).astype(_BF16)
                side.step(rg)
                if last:
                    for i, (p0, n, g0, g1) in enumerate(o_pieces):
                        if p0 + n - 1 == p and g1 - 1 == g:
                            @pl.when(j == NF - 1)
                            def _(i=i):
                                o_copy(i).start()

    def conv_step(j, carry):
        for cp in w_copies(j) + c_copies(j):
            cp.wait()
        for cp in w_copies(j + 1):
            cp.start()

        @pl.when(j + 1 < NU)
        def _():
            for cp in c_copies(j + 1):
                cp.start()

        side = _Side([(ln2_job(NB - 1, None), LN2_N), (kv_job(j), KV_N)], TPC * NG - 8)
        mlp_tile(j, 0, side)
        side.finish()
        sk = sk_ref[j]
        lhs = jnp.concatenate([sk[:, b * BLK:(b + 1) * BLK] for b in range(NB)], axis=0)
        kf = jnp.dot(lhs, fwd_ref[...], preferred_element_type=_F32)
        u = jnp.dot(kv_ref[oz].reshape(NB * CU, BLK).astype(_BF16), fwd_ref[...],
                    preferred_element_type=_F32)
        kf_ref[...] = kf.reshape(NB, CU, 2 * BLK)
        u_ref[...] = u.reshape(NB, CU, 2 * BLK)
        side = _Side([(mac_job(), MAC_N)], (NT - 1) * TPC * NG - 12)
        for t in range(1, NT):
            mlp_tile(j, t, side)
        side.finish()
        crow = pl.ds(pl.multiple_of(j * CU, CU), CU)
        hb = NB // 2
        for half in range(2):
            z = z_ref[oz, half * hb:(half + 1) * hb].reshape(hb * CU, 2 * BLK).astype(_BF16)
            y = jnp.dot(z, inv_ref[...], preferred_element_type=_F32)
            for bb in range(hb):
                b = half * hb + bb
                cols = slice(b * BLK, (b + 1) * BLK)
                yb = y[bb * CU:(bb + 1) * CU] + kv_ref[oz, b] * col_ref[4, crow, :]
                ga_ref[crow, cols] = q_ref[crow, cols].astype(_F32) * yb * g_ref[0:1, cols]
        return carry

    def plain_step(j, carry):
        for cp in w_copies(j):
            cp.wait()

        @pl.when(j + 1 < NF)
        def _():
            for cp in w_copies(j + 1):
                cp.start()

        for t in range(NT):
            mlp_tile(j, t, _Side([], 1), last=True)
        return carry

    with jax.named_scope('main'):
        lax.fori_loop(0, NU, conv_step, 0)
    with jax.named_scope('plain'):
        lax.fori_loop(NU, NF, plain_step, 0)
    for i in range(len(o_pieces)):
        o_copy(i).wait()


@jax.jit
def pallas_gated_mix__ssm_conv_h3__mixer_s_mlp__prompt_kernel(
    A_q: jax.Array,
    A_k: jax.Array,
    A_v: jax.Array,
    A_shift_k: jax.Array,
    A_ssm_k: jax.Array,
    A_ssm_D: jax.Array,
    B_x: jax.Array,
    B_w1: jax.Array,
    B_w2: jax.Array,
    B_w3: jax.Array,
    B_w4: jax.Array,
    gate_w: jax.Array,
):
    del B_x
    qT = A_q.reshape(S, D).T
    kT = A_k.reshape(S, D).T
    vT = A_v.reshape(S, D).T
    shT = A_shift_k.T
    w4T = B_w4.T
    fwd, inv = _dft_consts()
    fwd = jnp.asarray(fwd, _BF16)
    inv = jnp.asarray(inv, _BF16)

    hbm = pl.BlockSpec(memory_space=pl.ANY)

    outT = pl.pallas_call(
        _kernel,
        in_specs=[hbm] * 13,
        out_specs=hbm,
        out_shape=jax.ShapeDtypeStruct((D, S), _BF16),
        scratch_shapes=[
            pltpu.VMEM((D, S), _F32),
            pltpu.VMEM((D, S), _F32),
            pltpu.VMEM((2, D, TM), _F32),
            pltpu.VMEM((2, D, TM), _F32),
            pltpu.VMEM((S // 2, D), _U32),
            pltpu.VMEM((2, D, TM), _F32),
            pltpu.VMEM((2, D, TM), _F32),
            pltpu.VMEM((2, D, TM), _F32),
            pltpu.VMEM((2, D, TM), _F32),
            pltpu.VMEM((2, NB, CU, BLK), _F32),
            pltpu.VMEM((NB, CU, 2 * BLK), _F32),
            pltpu.VMEM((NB, CU, 2 * BLK), _F32),
            pltpu.VMEM((2, NB, CU, 2 * BLK), _F32),
            pltpu.VMEM((8, S), _F32),
            pltpu.VMEM((6, D, 128), _F32),
            pltpu.VMEM((D // 2, D), _U32),
            pltpu.VMEM((D // 2, D), _U32),
            pltpu.VMEM((D, S), _BF16),
            pltpu.VMEM((NU, CU, S), _BF16),
            pltpu.VMEM((NU, CU, S), _BF16),
            pltpu.VMEM((NU, CU, S), _BF16),
            pltpu.VMEM((D, D), _BF16),
            pltpu.VMEM((D, D), _BF16),
            pltpu.VMEM((NF, D, TF), _BF16),
            pltpu.VMEM((NF, D, TF), _BF16),
            pltpu.VMEM((D, S), _BF16),
            pltpu.VMEM((4, D), _BF16),
            pltpu.VMEM((D,), _BF16),
            pltpu.VMEM((D,), _BF16),
            pltpu.VMEM((BLK, 2 * BLK), _BF16),
            pltpu.VMEM((2 * BLK, BLK), _BF16),
            pltpu.VMEM((D + 8, BLK), _F32),
            pltpu.SemaphoreType.DMA((6,)),
        ],
        compiler_params=pltpu.CompilerParams(
            vmem_limit_bytes=110 * 1024 * 1024,
        ),
    )(qT, kT, vT, A_ssm_k, B_w1, B_w2, B_w3, w4T, shT, A_ssm_D, gate_w, fwd, inv)
    return outT.T.reshape(1, S, D)
```

```python
import numpy as np
import jax
import jax.numpy as jnp
from jax import lax
import jax.experimental.pallas as pl
import jax.experimental.pallas.tpu as pltpu

S, D, F = 2048, 576, 4608
BLK = 128
NB = S // BLK
TF = 512
NF = F // TF
TM = 512
NT = S // TM
TPC = TM // BLK
NU = 6
CU = D // NU
C4 = D // 4
RG = 16
NG = D // RG
KF = 512
W1P = ((0, 256), (256, D))
SHIFTS = (1, -1, 2, -2)
HF = 256
DH = D // 2
W2_ORDER = (0, 2, 1, 3)

_F32 = jnp.float32
_BF16 = jnp.bfloat16
_U32 = jnp.uint32


def _dft_consts():
    t = np.arange(BLK, dtype=np.float64)[:, None]
    f = np.arange(BLK, dtype=np.float64)[None, :]
    th = np.pi * (2.0 * f + 1.0) * t / (2.0 * BLK)
    fwd = np.concatenate([np.cos(th), -np.sin(th)], axis=1)
    inv = fwd.T / BLK
    return fwd.astype(_BF16), inv.astype(_BF16)


def _gelu(x):
    c = 0.7978845608028654
    t = jnp.tanh(x * (c + (c * 0.044715) * (x * x)))
    hx = 0.5 * x
    return hx + hx * t


def _col_bcast(row):
    return jnp.broadcast_to(row, (128, D)).T


def _fold8(x):
    acc = x[0:8]
    for r in range(1, x.shape[0] // 8):
        acc = acc + x[r * 8:(r + 1) * 8]
    return acc


def _pk(x):
    return pltpu.bitcast(x, _U32)


def _upk(x):
    return pltpu.bitcast(x, _BF16)


class _Side:
    def __init__(self, jobs, nslots, once=False):
        self.once = once
        self.jobs = []
        for gen, n in jobs:
            next(gen)
            self.jobs.append(gen)
        self.total = sum(n for _, n in jobs)
        self.nslots = nslots
        self.slot = 0
        self.done = 0

    def _one(self, dep):
        try:
            self.jobs[0].send(dep)
        except StopIteration:
            self.jobs.pop(0)
        self.done += 1

    def step(self, dep, weight=1):
        self.slot += weight
        target = min(self.total, -(-self.total * self.slot // self.nslots))
        while self.done < target:
            self._one(dep)
            if self.once:
                dep = None

    def finish(self):
        while self.done < self.total:
            self._one(None)
        assert not self.jobs


def _kernel(q_hbm, k_hbm, v_hbm, sk_hbm, w1_hbm, w2_hbm, w3_hbm, w4_hbm,
            sh_hbm, sd_hbm, gw_hbm, fwd_hbm, inv_hbm, o_hbm,
            acc_ref, ga_ref, xn1a_ref, xn1b_ref, xs_ref, xr_ref, xt_ref,
            g11_ref, g12_ref, g21_ref, g22_ref, sb_ref, h0_ref, h1_ref, h2_ref, h3_ref,
            kv_ref, u_ref, kf_ref, z_ref, g_ref, col_ref, w1t_ref, w2t_ref,
            q_ref, k_ref, v_ref, sk_ref, w1_ref, w2_ref, w3_ref, w4_ref, o_ref,
            sh_ref, sd_ref, gw_ref, fwd_ref, inv_ref,
            x1l_ref, sem):
    xn1_refs = (xn1a_ref, xn1b_ref)
    h_refs = (h0_ref, h1_ref, h2_ref, h3_ref)

    def copy(src, dst, s):
        return pltpu.make_async_copy(src, dst, sem.at[s])

    def q_copy(c):
        return copy(q_hbm.at[:, pl.ds(c * TM, TM)], q_ref.at[:, pl.ds(c * TM, TM)], (2, 3, 4, 4)[c])

    w1_copies = [copy(w1_hbm.at[r0:r1], w1_ref.at[r0:r1], s) for s, (r0, r1) in zip((1, NF), W1P)]
    par_copies = [copy(sh_hbm, sh_ref, 0), copy(sd_hbm, sd_ref, 0), copy(gw_hbm, gw_ref, 0)]

    def w3_copy(j, s):
        return copy(w3_hbm.at[:, pl.ds(j * TF, TF)], w3_ref.at[j], s)

    def w4_copy(j):
        return copy(w4_hbm.at[:, pl.ds(j * TF, TF)], w4_ref.at[j], j)

    def c_copies(j):
        rows = pl.ds(j * CU, CU)
        return [copy(k_hbm.at[rows, :], k_ref.at[j], j),
                copy(v_hbm.at[rows, :], v_ref.at[j], j),
                copy(sk_hbm.at[rows, :], sk_ref.at[j], j)]

    def step_copies(j):
        return ([w4_copy(j)] + ([w3_copy(j + 1, j)] if j + 1 < NF else [])
                + (c_copies(j) if j < NU else []))

    pre_copies = [copy(w2_hbm, w2_ref, NF), w3_copy(0, NF),
                  copy(fwd_hbm, fwd_ref, NF), copy(inv_hbm, inv_ref, NF)]

    o_pieces = [(0, D, c * TM, (c + 1) * TM) for c in range(NT - 1)]
    _c = (NT - 1) * TM
    o_pieces += [(DH, D, _c, _c + HF), (0, DH, _c + HF, S), (DH, D, _c + HF, S),
                 (0, 192, _c, _c + HF), (192, DH, _c, _c + HF)]

    def o_copy(i):
        r0, r1, c0, c1 = o_pieces[i]
        idx = (pl.ds(r0, r1 - r0), pl.ds(c0, c1 - c0))
        return copy(o_ref.at[idx], o_hbm.at[idx], 0)

    for cp in par_copies + [w1_copies[0]]:
        cp.start()
    later = ([q_copy(0), w1_copies[1], q_copy(1), q_copy(2), q_copy(3)] + pre_copies
             + step_copies(0) + step_copies(1))

    def start_next(n=1):
        for _ in range(n):
            if later:
                later.pop(0).start()

    lane = lax.broadcasted_iota(jnp.int32, (8, BLK), 1)
    sgn = 1.0 - 2.0 * (lane % 2).astype(_F32)
    never = sgn > 2.0
    oz = lax.fori_loop(0, 3, lambda i, c: c * i, 7)

    def pin(x, dep):
        if dep is None:
            return x
        d = dep[0:8]
        if x.dtype != d.dtype:
            d = pltpu.bitcast(d, x.dtype)
        head = jnp.where(never, d, x[0:8])
        return head if x.shape[0] == 8 else jnp.concatenate([head, x[8:]], axis=0)

    def sub_pinned(x, mu8, dep):
        m = pin(mu8, dep)
        return x - jnp.concatenate([m] * (x.shape[0] // 8), axis=0)

    def ln1_job(p):
        cols = slice(p * BLK, (p + 1) * BLK)
        ocols = slice((p % TPC) * BLK, (p % TPC + 1) * BLK)
        R = 2 * RG
        s = None
        for g in range(D // (2 * R)):
            dep = yield
            a = _fold8(pin(q_ref[g * 2 * R:(g + 1) * 2 * R, cols].astype(_F32), dep))
            s = a if s is None else s + a
        mu = jnp.broadcast_to(jnp.sum(s, axis=0, keepdims=True) * (1.0 / D), (8, BLK))
        v = None
        for g in range(D // R):
            dep = yield
            xc = sub_pinned(q_ref[g * R:(g + 1) * R, cols].astype(_F32), mu, dep)
            a = _fold8(xc * xc)
            v = a if v is None else v + a
        rs = lax.rsqrt(jnp.sum(v, axis=0, keepdims=True) * (1.0 / D) + 1e-5)
        for g in range(D // R):
            dep = yield
            xc = sub_pinned(q_ref[g * R:(g + 1) * R, cols].astype(_F32), mu, dep)
            xn1_refs[(p // TPC) % 2][0, g * R:(g + 1) * R, ocols] = xc * rs

    LN1_N = D // (4 * RG) + 2 * (D // (2 * RG))

    def ln2_job(p, s):
        if s is None:
            src, cols = x1l_ref, slice(0, BLK)
            s = x1l_ref[D:D + 8, :]
        else:
            src, cols = acc_ref, slice(p * BLK, (p + 1) * BLK)
        R = 2 * RG
        mu = None
        v = None
        for g in range(D // R):
            dep = yield
            if mu is None:
                mu = jnp.broadcast_to(jnp.sum(s, axis=0, keepdims=True) * (1.0 / D), (8, BLK))
            xc = sub_pinned(src[g * R:(g + 1) * R, cols], mu, dep)
            a = _fold8(xc * xc)
            v = a if v is None else v + a
        rs = lax.rsqrt(jnp.sum(v, axis=0, keepdims=True) * (1.0 / D) + 1e-5)
        t = p % TPC
        for g in range(D // R):
            dep = yield
            xt_ref[0, t, g * R:(g + 1) * R, :] = sub_pinned(
                src[g * R:(g + 1) * R, cols], mu, dep) * rs
        pair = (p // TPC) * 2 + t % 2
        prow = slice(pair * (BLK // 2), (pair + 1) * (BLK // 2))

        def blk(tt, half, k):
            r0 = half * HF + k * BLK
            return xt_ref[oz, tt, r0:r0 + BLK, :]

        if t < 2:
            ops = [(2, (t, 0), None, 1), (4, (t, 0), (t, 1), 1)]
        else:
            ops = [(3, (t, 1), None, 1), (1, (t, 0), (t, 1), 1), (0, (t - 2, 0), (t, 1), 1),
                   (5, (t, 0), (t - 2, 0), -1), (6, (t - 2, 1), (t, 1), -1)]
        for idx, a, b, sign in ops:
            for k in range(2):
                dep = yield
                x = pin(blk(a[0], a[1], k), dep)
                if b is not None:
                    x = x + blk(b[0], b[1], k) if sign > 0 else x - blk(b[0], b[1], k)
                xs_ref[idx, prow, k * BLK:(k + 1) * BLK] = _pk(x.astype(_BF16).T)
        dep = yield
        x = pin(xt_ref[oz, t, KF:D, :], dep)
        xr_ref[p * (BLK // 2):(p + 1) * (BLK // 2), :] = _pk(x.astype(_BF16).T)

    def ln2_n(p):
        return 2 * (D // (2 * RG)) + (5 if p % TPC < 2 else 11)

    def sb_job(j, which=range(5)):
        terms = [((0, 0), (1, 1), 1), ((0, 1), (1, 1), -1), ((1, 0), (0, 0), -1),
                 ((0, 0), (0, 1), 1), ((1, 0), (1, 1), 1)]
        for i in which:
            a, b, sign = terms[i]
            for g in range(HF // RG):
                dep = yield

                def blk(rc):
                    r0 = rc[0] * HF + g * RG
                    return w3_ref[j, r0:r0 + RG, rc[1] * HF:(rc[1] + 1) * HF].astype(_F32)

                x = blk(a)
                x = jnp.concatenate([pin(x[:, 0:BLK], dep), x[:, BLK:]], axis=1)
                x = x + blk(b) if sign > 0 else x - blk(b)
                sb_ref[i, g * 8:(g + 1) * 8, :] = _pk(x.astype(_BF16))

    SB_N = 5 * (HF // RG)

    def kv_job(j):
        for g in range(CU // RG):
            rows = slice(g * RG, (g + 1) * RG)
            crow = pl.ds(pl.multiple_of(j * CU + g * RG, RG), RG)
            prev = None
            for b in range(NB):
                dep = yield
                cols = slice(b * BLK, (b + 1) * BLK)
                ku = pin(_pk(k_ref[j, rows, cols]), dep)
                rolled = [pltpu.roll(ku, tau, 1) for tau in range(1, 4)]
                ks = _upk(ku).astype(_F32) * col_ref[0, crow, :]
                for tau in range(1, 4):
                    lo = jnp.zeros_like(ku) if prev is None else prev[tau - 1]
                    sh = _upk(jnp.where(lane < tau, lo, rolled[tau - 1])).astype(_F32)
                    ks = ks + sh * col_ref[tau, crow, :]
                prev = rolled
                kv_ref[0, b, rows, :] = ks * v_ref[j, rows, cols].astype(_F32)

    KV_N = (CU // RG) * NB

    def mac_job():
        for g in range(CU // 8):
            rows = slice(g * 8, (g + 1) * 8)
            yp = None
            for i in range(NB):
                yr = None
                yi = None
                for m in range(i + 1):
                    dep = yield
                    kr = pin(kf_ref[m, rows, 0:BLK], dep)
                    ki = kf_ref[m, rows, BLK:2 * BLK]
                    ur = u_ref[i - m, rows, 0:BLK]
                    ui = u_ref[i - m, rows, BLK:2 * BLK]
                    pr = kr * ur - ki * ui
                    pi = kr * ui + ki * ur
                    yr = pr if yr is None else yr + pr
                    yi = pi if yi is None else yi + pi
                if yp is None:
                    zr, zi = yr, yi
                else:
                    zr = yr - sgn * yp[1]
                    zi = yi + sgn * yp[0]
                yp = (yr, yi)
                z_ref[0, i, rows, 0:BLK] = zr
                z_ref[0, i, rows, BLK:2 * BLK] = zi

    MAC_N = (CU // 8) * (NB * (NB + 1) // 2)

    start_next()
    with jax.named_scope('setup'):
        for cp in par_copies:
            cp.wait()
        start_next()
        col_ref[5] = _col_bcast(gw_ref[...].astype(_F32).reshape(1, D))
        for r in range(4):
            col_ref[r] = _col_bcast(sh_ref[r:r + 1, :].astype(_F32))
        col_ref[4] = _col_bcast(sd_ref[...].astype(_F32).reshape(1, D))
        w1_copies[0].wait()
        start_next()
        w1t_ref[:, W1P[0][0]:W1P[0][1]] = _pk(w1_ref[W1P[0][0]:W1P[0][1], :].T)
    with jax.named_scope('setup2'):
        q_copy(0).wait()
        start_next()
        _Side([(ln1_job(p), LN1_N) for p in range(3)], 1).finish()
    with jax.named_scope('setup3'):
        w1_copies[1].wait()
        start_next(1)
        w1t_ref[:, W1P[1][0]:W1P[1][1]] = _pk(w1_ref[W1P[1][0]:W1P[1][1], :].T)
        _Side([(ln1_job(3), LN1_N)], 1).finish()

    def w_segment(wt_ref, x_tile, c, per_round, epilogue, order=range(TPC)):
        side, wgt, fin = per_round(0)
        xr = jnp.concatenate([x_tile(KF, D, c * TPC + t) for t in range(TPC)], axis=1)
        part = jnp.dot(_upk(wt_ref[:, KF:D]), xr.astype(_BF16), preferred_element_type=_F32)
        for g in range(NG):
            side.step(part[g * RG:(g + 1) * RG, 0:BLK], wgt)
        if fin:
            side.finish()
        for rnd, t in enumerate(order):
            p = c * TPC + t
            side, wgt, fin = per_round(rnd + 1)
            r = jnp.dot(_upk(wt_ref[:, 0:KF]), x_tile(0, KF, p).astype(_BF16),
                        preferred_element_type=_F32)
            for g in range(NG):
                rg = r[g * RG:(g + 1) * RG] + part[g * RG:(g + 1) * RG, t * BLK:(t + 1) * BLK]
                epilogue(rg, g, p)
                side.step(rg, wgt)
            if fin:
                side.finish()

    def w1_epilogue(rg, g, p):
        sft = SHIFTS[g * RG // C4]
        h_refs[p // TPC][0, g * RG:(g + 1) * RG, (p % TPC) * BLK:(p % TPC + 1) * BLK] = (
            pltpu.roll(_gelu(rg), sft % BLK, 1))

    def xn1_tile(r0, r1, p):
        return xn1_refs[(p // TPC) % 2][oz, r0:r1, (p % TPC) * BLK:(p % TPC + 1) * BLK]

    def h_tile(r0, r1, p):
        if p < 0 or p >= NB:
            return jnp.zeros((r1 - r0, BLK), _F32)
        return h_refs[p // TPC][oz, r0:r1, (p % TPC) * BLK:(p % TPC + 1) * BLK]

    def hs_tile(r0, r1, p):
        parts = []
        for gi, sft in enumerate(SHIFTS):
            a0, a1 = max(r0, gi * C4), min(r1, (gi + 1) * C4)
            if a0 >= a1:
                continue
            ln = lax.broadcasted_iota(jnp.int32, (a1 - a0, BLK), 1)
            if sft > 0:
                parts.append(jnp.where(ln < sft, h_tile(a0, a1, p - 1), h_tile(a0, a1, p)))
            else:
                parts.append(jnp.where(ln >= BLK + sft, h_tile(a0, a1, p + 1), h_tile(a0, a1, p)))
        return parts[0] if len(parts) == 1 else jnp.concatenate(parts, axis=0)

    with jax.named_scope('w1'):
        for c in range(NT):
            state = {}

            def per_round(rnd, c=c, state=state):
                first = 1 if c < 2 else 0
                if c == NT - 1 and rnd == 1:
                    for j in range(2, NF):
                        for cp in step_copies(j):
                            cp.start()
                    for cp in pre_copies:
                        cp.wait()
                    w2t_ref[...] = _pk(w2_ref[...].T)
                if rnd < first or c + 1 == NT:
                    return _Side([], 1), 1, False
                if rnd == first:
                    if c == 0:
                        q_copy(1).wait()
                    if c == 1:
                        start_next(len(later))
                        q_copy(2).wait()
                        q_copy(3).wait()
                    jobs = [(ln1_job((c + 1) * TPC + t), LN1_N) for t in range(TPC)]
                    state['side'] = _Side(jobs, (4 if c < 2 else 6) * NG - 16)
                return state['side'], (2 if rnd == 0 else 1), rnd == TPC

            w_segment(w1t_ref, xn1_tile, c, per_round, w1_epilogue)

    sums = {}
    gsums = {}

    def w2_epilogue(rg, g, p):
        cols = slice(p * BLK, (p + 1) * BLK)
        x = q_ref[g * RG:(g + 1) * RG, cols].astype(_F32)
        x1 = rg + x
        acc_ref[g * RG:(g + 1) * RG, cols] = x1
        if p == NB - 1:
            x1l_ref[g * RG:(g + 1) * RG, :] = x1
        a = _fold8(x1)
        b = _fold8(x * col_ref[5, g * RG:(g + 1) * RG, :])
        sums[p] = a if g == 0 else sums[p] + a
        gsums[p] = b if g == 0 else gsums[p] + b
        if g == NG - 1:
            gate = jax.nn.sigmoid(jnp.sum(gsums.pop(p), axis=0, keepdims=True))
            g_ref[:, cols] = jnp.broadcast_to(gate, (8, BLK))

    with jax.named_scope('w2'):
        for c in range(NT):
            def per_round(rnd, c=c):
                pprev = c * TPC + W2_ORDER[rnd - 2] if rnd >= 2 else c * TPC - 1 if rnd == 0 else -1
                jobs = [(ln2_job(pprev, sums.pop(pprev)), ln2_n(pprev))] if pprev >= 0 else []
                if c == 0 and rnd < 2:
                    jobs.append((sb_job(0, (0, 1, 2) if rnd == 0 else (3, 4)),
                                 (3 if rnd == 0 else 2) * (HF // RG)))
                return _Side(jobs, 26 if (c, rnd) == (NT - 1, TPC) else NG), 1, True
            w_segment(w2t_ref, hs_tile, c, per_round, w2_epilogue, W2_ORDER)
        x1l_ref[D:D + 8, :] = sums.pop(NB - 1)
        assert not later

    def weight_sums(j):
        f = lambda x: x.astype(_F32)
        b = lambda x: x.astype(_BF16)
        sb = [_upk(sb_ref[0]), w3_ref[j, 0:HF, 0:HF], _upk(sb_ref[1]), _upk(sb_ref[2]),
              w3_ref[j, HF:KF, HF:TF], _upk(sb_ref[3]), _upk(sb_ref[4])]
        a11, a12 = w4_ref[j, 0:DH, 0:HF], w4_ref[j, 0:DH, HF:TF]
        a21, a22 = w4_ref[j, DH:D, 0:HF], w4_ref[j, DH:D, HF:TF]
        sa = [b(f(a11) + f(a22)), b(f(a21) + f(a22)), a11, a22, b(f(a11) + f(a12)),
              b(f(a21) - f(a11)), b(f(a12) - f(a22))]
        return sb, sa

    def mlp_tile(j, t, ws, side, side2=None, last=False):
        sb, sa = ws

        def feed(val, wgt):
            for g in range(val.shape[0] // RG):
                side.step(val[g * RG:(g + 1) * RG, 0:BLK], wgt)
            return val

        def m(i, wgt):
            x = _upk(xs_ref[i - 1, t * (HF // 2):(t + 1) * (HF // 2), :])
            return feed(jnp.dot(x, sb[i - 1], preferred_element_type=_F32), wgt)

        def rem(half):
            rows = slice(t * HF + half * (HF // 2), t * HF + (half + 1) * (HF // 2))
            return feed(jnp.dot(_upk(xr_ref[rows, :]), w3_ref[j, KF:D, :],
                                preferred_element_type=_F32), W_REM)

        def n(i, x, wgt):
            val = feed(lax.dot_general(sa[i - 1], x.astype(_BF16), (((1,), (1,)), ((), ())),
                                       preferred_element_type=_F32), wgt)
            if isinstance(side2, _Side):
                for g in range(DH // RG):
                    side2.step(val[g * RG:(g + 1) * RG, BLK:2 * BLK])
            return val

        def add(r0, c0, val):
            cols = slice(t * TM + c0, t * TM + c0 + HF)
            for g in range(DH // RG):
                rows = slice(r0 + g * RG, r0 + (g + 1) * RG)
                a = acc_ref[rows, cols] + val[g * RG:(g + 1) * RG]
                acc_ref[rows, cols] = a
                if last:
                    omg = jnp.concatenate([1.0 - g_ref[:, cols]] * 2, axis=0)
                    o_ref[rows, cols] = (ga_ref[rows, cols] + omg * a).astype(_BF16)
                    for i, (p0, p1, q0, q1) in enumerate(o_pieces):
                        if t < NT - 1:
                            hit = i == t and r0 == 0 and c0 == 0 and g == DH // RG - 1
                        else:
                            hit = i >= NT - 1 and q0 == cols.start and p1 == rows.stop
                        if hit:
                            @pl.when(j == NF - 1)
                            def _(i=i):
                                o_copy(i).start()

        ra = rem(0)
        m5 = m(5, W_LIGHT)
        m3 = m(3, W_GELU)
        g12_ref[0] = _gelu(ra[:, HF:TF] + m3 + m5)
        m4 = m(4, W_LIGHT)
        m1 = m(1, W_LIGHT)
        m7 = m(7, W_GELU)
        g11_ref[0] = _gelu(ra[:, 0:HF] + m1 + m4 - m5 + m7)
        rb = rem(1)
        m2 = m(2, W_GELU)
        g21_ref[0] = _gelu(rb[:, 0:HF] + m2 + m4)
        n4 = n(4, g12_ref[oz] - g11_ref[oz], W_MID)
        m6 = m(6, W_GELU)
        g22_ref[0] = _gelu(rb[:, HF:TF] + m1 - m2 + m3 + m6)
        if side2 is not None:
            side2 = side2()
        n2 = n(2, g11_ref[oz], W_MID)
        add(DH, 0, n2 + n4)
        n6 = n(6, g11_ref[oz] + g21_ref[oz], W_MID)
        n5 = n(5, g22_ref[oz], W_MID)
        n3 = n(3, g21_ref[oz] - g22_ref[oz], W_MID)
        add(0, HF, n3 + n5)
        n1 = n(1, g11_ref[oz] + g22_ref[oz], W_MID)
        add(DH, HF, n1 - n2 + n3 + n6)
        n7 = n(7, g12_ref[oz] + g22_ref[oz], W_MID)
        add(0, 0, n1 + n4 - n5 + n7)
        if side2 is not None:
            side2.finish()

    W_REM, W_LIGHT, W_GELU, W_MID = 1, 3, 0, 2
    TILE_W = 32 * W_REM + 3 * 16 * W_LIGHT + 4 * 16 * W_GELU + 7 * 18 * W_MID

    def conv_step(j, carry):
        for cp in [w4_copy(j), w3_copy(j + 1, j)] + c_copies(j):
            cp.wait()
        ws = weight_sums(j)
        side = _Side([(ln2_job(NB - 1, None), ln2_n(NB - 1)), (kv_job(j), KV_N)], TILE_W - 30)
        mlp_tile(j, 0, ws, side)
        side.finish()
        sk = sk_ref[j]
        lhs = jnp.concatenate([sk[:, b * BLK:(b + 1) * BLK] for b in range(NB)], axis=0)
        kf = jnp.dot(lhs, fwd_ref[...], preferred_element_type=_F32)
        u = jnp.dot(kv_ref[oz].reshape(NB * CU, BLK).astype(_BF16), fwd_ref[...],
                    preferred_element_type=_F32)
        kf_ref[...] = kf.reshape(NB, CU, 2 * BLK)
        u_ref[...] = u.reshape(NB, CU, 2 * BLK)
        side = _Side([(mac_job(), MAC_N)], (NT - 1) * TILE_W - 30, once=True)
        side2 = lambda: _Side([(sb_job(j + 1), SB_N)], 6 * (DH // RG) - 10)
        for t in range(1, NT):
            mlp_tile(j, t, ws, side, side2 if t == NT - 1 else None)
        side.finish()
        crow = pl.ds(pl.multiple_of(j * CU, CU), CU)
        hb = NB // 2
        for half in range(2):
            z = z_ref[oz, half * hb:(half + 1) * hb].reshape(hb * CU, 2 * BLK).astype(_BF16)
            y = jnp.dot(z, inv_ref[...], preferred_element_type=_F32)
            for bb in range(hb):
                b = half * hb + bb
                cols = slice(b * BLK, (b + 1) * BLK)
                yb = y[bb * CU:(bb + 1) * CU] + kv_ref[oz, b] * col_ref[4, crow, :]
                ga_ref[crow, cols] = q_ref[crow, cols].astype(_F32) * yb * g_ref[0:1, cols]
        return carry

    def plain_step(j, carry):
        w4_copy(j).wait()

        @pl.when(j + 1 < NF)
        def _():
            w3_copy(j + 1, j).wait()

        ws = weight_sums(j)
        side2 = lambda: _Side([(sb_job(jnp.minimum(j + 1, NF - 1)), SB_N)], 6 * (DH // RG) - 10)
        for t in range(NT):
            mlp_tile(j, t, ws, _Side([], 1), side2 if t == NT - 1 else None, last=True)
        return carry

    with jax.named_scope('main'):
        lax.fori_loop(0, NU, conv_step, 0)
    with jax.named_scope('plain'):
        lax.fori_loop(NU, NF, plain_step, 0)
    for i in range(len(o_pieces)):
        o_copy(i).wait()


@jax.jit
def pallas_gated_mix__ssm_conv_h3__mixer_s_mlp__prompt_kernel(
    A_q: jax.Array,
    A_k: jax.Array,
    A_v: jax.Array,
    A_shift_k: jax.Array,
    A_ssm_k: jax.Array,
    A_ssm_D: jax.Array,
    B_x: jax.Array,
    B_w1: jax.Array,
    B_w2: jax.Array,
    B_w3: jax.Array,
    B_w4: jax.Array,
    gate_w: jax.Array,
):
    del B_x
    qT = A_q.reshape(S, D).T
    kT = A_k.reshape(S, D).T
    vT = A_v.reshape(S, D).T
    shT = A_shift_k.T
    w4T = B_w4.T
    fwd, inv = _dft_consts()

    hbm = pl.BlockSpec(memory_space=pl.ANY)

    outT = pl.pallas_call(
        _kernel,
        in_specs=[hbm] * 13,
        out_specs=hbm,
        out_shape=jax.ShapeDtypeStruct((D, S), _BF16),
        scratch_shapes=[
            pltpu.VMEM((D, S), _F32),
            pltpu.VMEM((D, S), _F32),
            pltpu.VMEM((2, D, TM), _F32),
            pltpu.VMEM((2, D, TM), _F32),
            pltpu.VMEM((7, S // 4, HF), _U32),
            pltpu.VMEM((S // 2, D - KF), _U32),
            pltpu.VMEM((2, TPC, D, BLK), _F32),
            pltpu.VMEM((2, HF, HF), _F32),
            pltpu.VMEM((2, HF, HF), _F32),
            pltpu.VMEM((2, HF, HF), _F32),
            pltpu.VMEM((2, HF, HF), _F32),
            pltpu.VMEM((5, HF // 2, HF), _U32),
            pltpu.VMEM((2, D, TM), _F32),
            pltpu.VMEM((2, D, TM), _F32),
            pltpu.VMEM((2, D, TM), _F32),
            pltpu.VMEM((2, D, TM), _F32),
            pltpu.VMEM((2, NB, CU, BLK), _F32),
            pltpu.VMEM((NB, CU, 2 * BLK), _F32),
            pltpu.VMEM((NB, CU, 2 * BLK), _F32),
            pltpu.VMEM((2, NB, CU, 2 * BLK), _F32),
            pltpu.VMEM((8, S), _F32),
            pltpu.VMEM((6, D, 128), _F32),
            pltpu.VMEM((D // 2, D), _U32),
            pltpu.VMEM((D // 2, D), _U32),
            pltpu.VMEM((D, S), _BF16),
            pltpu.VMEM((NU, CU, S), _BF16),
            pltpu.VMEM((NU, CU, S), _BF16),
            pltpu.VMEM((NU, CU, S), _BF16),
            pltpu.VMEM((D, D), _BF16),
            pltpu.VMEM((D, D), _BF16),
            pltpu.VMEM((NF, D, TF), _BF16),
            pltpu.VMEM((NF, D, TF), _BF16),
            pltpu.VMEM((D, S), _BF16),
            pltpu.VMEM((4, D), _BF16),
            pltpu.VMEM((D,), _BF16),
            pltpu.VMEM((D,), _BF16),
            pltpu.VMEM((BLK, 2 * BLK), _BF16),
            pltpu.VMEM((2 * BLK, BLK), _BF16),
            pltpu.VMEM((D + 8, BLK), _F32),
            pltpu.SemaphoreType.DMA((NF + 1,)),
        ],
        compiler_params=pltpu.CompilerParams(
            vmem_limit_bytes=110 * 1024 * 1024,
        ),
    )(qT, kT, vT, A_ssm_k, B_w1, B_w2, B_w3, w4T, shT, A_ssm_D, gate_w, fwd, inv)
    return outT.T.reshape(1, S, D)
```
